```python
import os as _os
_os.environ.setdefault("JAX_PLATFORMS", "cpu")
import jax
import jax.numpy as jnp

def _softmax(x, axis=-1):
    return jax.nn.softmax(x, axis=axis)
def _gelu(x):
    return jax.nn.gelu(x, approximate=True)
def _silu(x):
    return jax.nn.silu(x)
def _sigmoid(x):
    return jax.nn.sigmoid(x)
def _layernorm(x, axis=-1, eps=1e-5):
    m = jnp.mean(x, axis=axis, keepdims=True)
    v = jnp.var(x, axis=axis, keepdims=True)
    return (x - m) / jnp.sqrt(v + eps)
def _scatter_add(tgt, idx, src, axis=0):
    return tgt.at[idx].add(src)
def _segment_sum(src, seg, n):
    return jax.ops.segment_sum(src, seg, n)
class _Rng:
    def __init__(self, key):
        self._k = key
    def _next(self):
        self._k, sub = jax.random.split(self._k)
        return sub
    def normal(self, shape):
        return jax.random.normal(self._next(), shape, dtype=jnp.bfloat16)
    def randint(self, lo, hi, shape):
        return jax.random.randint(self._next(), shape, lo, hi, dtype=jnp.int32)
    def uniform(self, shape, lo=0.0, hi=1.0):
        return jax.random.uniform(self._next(), shape, jnp.bfloat16, lo, hi)
    def permutation(self, n):
        return jax.random.permutation(self._next(), n)


kernel_name = 'sequential_preLN__linear_attn_block__dense_activation_squared_relu__prompt'

def setup_inputs():
    _rng = _Rng(jax.random.key(int.from_bytes(__import__("os").urandom(4), "little")))
    _w = (lambda a: (lambda t: t.astype(jnp.bfloat16) if jnp.issubdtype(t.dtype, jnp.floating) else t)(jnp.asarray(a)))
    def _A_setup():
        B, S, D = 1, 2048, 576
        return {
            "x": _w((lambda *s: _rng.normal(s) * 0.05)(B, S, D)),
            "wqkv": _w((lambda *s: _rng.normal(s) * 0.1)(D, 3 * D)),
            "wo": _w((lambda *s: _rng.normal(s) * 0.05)(D, D)),
        }
    _A_in = _A_setup()

    def _B_setup():
        B, S, D, F = 1, 2048, 576, 4608
        return {
            "x": _w((lambda *s: _rng.normal(s) * 0.05)(B, S, D)),
            "w1": _w((lambda *s: _rng.normal(s) * 0.05)(D, F)),
            "b1": _w((lambda *s: _rng.normal(s) * 0.05)(F)),
            "w2": _w((lambda *s: _rng.normal(s) * 0.05)(F, D)),
            "b2": _w((lambda *s: _rng.normal(s) * 0.05)(D)),
        }
    _B_in = _B_setup()

    return {
        "A_x": _A_in["x"],
        "A_wqkv": _A_in["wqkv"],
        "A_wo": _A_in["wo"],
        "B_x": _B_in["x"],
        "B_w1": _B_in["w1"],
        "B_b1": _B_in["b1"],
        "B_w2": _B_in["w2"],
        "B_b2": _B_in["b2"],
    }

def reference(A_x, A_wqkv, A_wo, B_x, B_w1, B_b1, B_w2, B_b2):
    def _A_ref(x, wqkv, wo):
        B, S, D = x.shape
        H = 32; Dh = D // H
        qkv = (lambda x, *d: x.transpose(*d))((x @ wqkv).reshape(B, S, 3, H, Dh), 2, 0, 3, 1, 4)
        q, k, v = qkv[0], qkv[1], qkv[2]
        phi = lambda t: jnp.where(t > 0, t + 1, jnp.exp(t)) + 1e-6
        pq, pk = phi(q), phi(k)
        kv = jnp.einsum("bhsd,bhse->bhde", pk, v)
        z = jnp.einsum("bhsd->bhd", pk)
        num = jnp.einsum("bhqd,bhde->bhqe", pq, kv)
        den = jnp.einsum("bhqd,bhd->bhq", pq, z)[..., None] + 1e-6
        o = num / den
        return (lambda x, *d: x.transpose(*d))(o, 0, 2, 1, 3).reshape(B, S, D) @ wo

    def _B_ref(x, w1, b1, w2, b2):
        h = jnp.einsum("bsd,df->bsf", x, w1) + b1
        zero = jnp.zeros_like(h)
        r = jnp.where(h > zero, h, zero)
        h = r * r
        out = jnp.einsum("bsf,fd->bsd", h, w2) + b2
        return out

    x = A_x
    h = x + _A_ref(_layernorm(x, axis=-1), A_wqkv, A_wo)
    h2 = h + _B_ref(_layernorm(h, axis=-1), B_w1, B_b1, B_w2, B_b2)
    return h2
```

```python
import functools
import jax
import jax.numpy as jnp
from jax import lax
import jax.experimental.pallas as pl
import jax.experimental.pallas.tpu as pltpu

S, D, F, H = 2048, 576, 4608, 32
DH = D // H
DA = D + 16
bf16, f32 = jnp.bfloat16, jnp.float32
NN = (((1,), (0,)), ((), ()))
NT = (((1,), (1,)), ((), ()))
TN = (((0,), (0,)), ((), ()))


def _dot(a, b, dims=NN):
    return lax.dot_general(a, b, dims, preferred_element_type=f32)


def _phi(t):
    return jnp.where(t > 0, t + 1.0, jnp.exp(t)) + 1e-6


def _ln_cols(x):
    m = jnp.sum(x, axis=0, keepdims=True) * (1.0 / D)
    xc = x - m
    v = jnp.sum(xc * xc, axis=0, keepdims=True) * (1.0 / D)
    return xc * lax.rsqrt(v + 1e-5)


def _head_of(i):
    return (i * 3641) >> 16


def make(T=512, TF=512):
    NT_ = S // T

    def kernel(x_hbm, wqkv_hbm, wo_hbm, w1_hbm, b1_hbm, w2_hbm, b2_hbm, o_hbm,
               x_v, wqkv_v, wo_v, w1_v, w2_v, b1_v, b2_v,
               xn_v, pq_v, h_v, hn_v, o_v, sems):
        cp_x = pltpu.make_async_copy(x_hbm, x_v, sems.at[0])
        cp_wqkv = pltpu.make_async_copy(wqkv_hbm, wqkv_v, sems.at[1])
        cp_wo = pltpu.make_async_copy(wo_hbm, wo_v, sems.at[2])
        cp_w1 = pltpu.make_async_copy(w1_hbm, w1_v.at[pl.ds(0, D), :], sems.at[3])
        cp_w2 = pltpu.make_async_copy(w2_hbm, w2_v, sems.at[4])
        cp_b1 = pltpu.make_async_copy(b1_hbm, b1_v, sems.at[5])
        cp_b2 = pltpu.make_async_copy(b2_hbm, b2_v, sems.at[6])
        cp_x.start(); cp_wqkv.start(); cp_b1.start(); cp_b2.start()
        cp_x.wait(); cp_wqkv.wait()
        cp_wo.start(); cp_w1.start(); cp_w2.start()

        row16 = lax.broadcasted_iota(jnp.int32, (16, T), 0)
        ones_rows = jnp.where(row16 == 0, 1.0, 0.0).astype(bf16)

        G = jnp.zeros((DA, D), f32)
        for t in range(NT_):
            sl = pl.ds(t * T, T)
            xn = _ln_cols(x_v[:, sl].astype(f32)).astype(bf16)
            xn_v[0:D, sl] = xn
            xn_v[D:DA, sl] = ones_rows
            k = _dot(wqkv_v[:, D:2 * D], xn, TN)
            pk = _phi(k).astype(bf16)
            G = G + _dot(xn_v[:, sl], pk, NT)

        Gb = G[0:D, :].astype(bf16)
        z = G[D:D + 1, :]
        ri = lax.broadcasted_iota(jnp.int32, (D, D), 0)
        ci = lax.broadcasted_iota(jnp.int32, (D, D), 1)
        same = _head_of(ri) == _head_of(ci)
        kv = _dot(Gb, wqkv_v[:, 2 * D:3 * D], TN)
        kvm = jnp.where(same, kv, 0.0).astype(bf16)
        zexp = jnp.where(same, z, 0.0).astype(bf16)
        cp_wo.wait()
        w2att = _dot(kvm, wo_v[...]).astype(bf16)

        for t in range(NT_):
            sl = pl.ds(t * T, T)
            q = _dot(wqkv_v[:, 0:D], xn_v[0:D, sl], TN)
            pq = _phi(q)
            pqb = pq.astype(bf16)
            den = _dot(zexp, pqb) + 1e-6
            pq_v[:, sl] = (pqb.astype(f32) / den).astype(bf16)

        cp_b1.wait(); cp_b2.wait()
        r16 = lax.broadcasted_iota(jnp.int32, (16, 128), 0)
        b1f = b1_v[...].astype(f32)
        for i in range(F // 128):
            w1_v[D:DA, i * 128:(i + 1) * 128] = jnp.where(r16 == 0, b1f[i:i + 1, :], 0.0).astype(bf16)
        b2row = b2_v[...].reshape(1, D).astype(f32)
        r16d = lax.broadcasted_iota(jnp.int32, (16, D), 0)
        b2t = jnp.where(r16d == 0, b2row, 0.0).astype(bf16)
        b2col = _dot(b2t, jnp.ones((16, 128), bf16), TN)

        for t in range(NT_):
            sl = pl.ds(t * T, T)
            h = x_v[:, sl].astype(f32) + _dot(w2att, pq_v[:, sl], TN)
            hn_v[0:D, sl] = _ln_cols(h).astype(bf16)
            hn_v[D:DA, sl] = ones_rows
            for j in range(T // 128):
                h_v[:, t * T + j * 128:t * T + (j + 1) * 128] = h[:, j * 128:(j + 1) * 128] + b2col

        cp_w1.wait(); cp_w2.wait()

        def ffn(t, c):
            sl = pl.ds(pl.multiple_of(t * TF, TF), TF)
            hh = _dot(w1_v[...], hn_v[:, sl], TN)
            r = jnp.maximum(hh, 0.0)
            r = (r * r).astype(bf16)
            o = h_v[:, sl] + _dot(w2_v[...], r)
            o_v[:, sl] = o.astype(bf16)
            return c
        lax.fori_loop(0, S // TF, ffn, 0)
        cp_o = pltpu.make_async_copy(o_v, o_hbm, sems.at[7])
        cp_o.start(); cp_o.wait()

    def fn(A_x, A_wqkv, A_wo, B_x, B_w1, B_b1, B_w2, B_b2):
        del B_x
        xt = A_x.reshape(S, D).T
        w2t = B_w2.T
        b1 = B_b1.reshape(F // 128, 128)
        anyspec = pl.BlockSpec(memory_space=pl.ANY)
        out = pl.pallas_call(
            kernel,
            out_shape=jax.ShapeDtypeStruct((D, S), bf16),
            in_specs=[anyspec] * 7,
            out_specs=anyspec,
            scratch_shapes=[
                pltpu.VMEM((D, S), bf16), pltpu.VMEM((D, 3 * D), bf16), pltpu.VMEM((D, D), bf16),
                pltpu.VMEM((DA, F), bf16), pltpu.VMEM((D, F), bf16),
                pltpu.VMEM((F // 128, 128), bf16), pltpu.VMEM((D,), bf16),
                pltpu.VMEM((DA, S), bf16), pltpu.VMEM((D, S), bf16), pltpu.VMEM((D, S), f32),
                pltpu.VMEM((DA, S), bf16), pltpu.VMEM((D, S), bf16),
                pltpu.SemaphoreType.DMA((8,)),
            ],
            compiler_params=pltpu.CompilerParams(vmem_limit_bytes=100 * 2**20),
            name="v1",
        )(xt, A_wqkv, A_wo, B_w1, b1, w2t, B_b2)
        return out.T.reshape(1, S, D)
    return fn


_fn = make(512, 512)


@jax.jit
def pallas_sequential_preLN__linear_attn_block__dense_activation_squared_relu__prompt_kernel(
    A_x: jax.Array,
    A_wqkv: jax.Array,
    A_wo: jax.Array,
    B_x: jax.Array,
    B_w1: jax.Array,
    B_b1: jax.Array,
    B_w2: jax.Array,
    B_b2: jax.Array,
):
    return _fn(A_x, A_wqkv, A_wo, B_x, B_w1, B_b1, B_w2, B_b2)
```

```python
import jax
import jax.numpy as jnp
from jax import lax
import jax.experimental.pallas as pl
import jax.experimental.pallas.tpu as pltpu

S, D, F, H = 2048, 576, 4608, 32
DH = D // H
DA = D + 16
FH, FQ, DHF = F // 2, F // 4, D // 2
T = 512
TH = T // 2
NTI = S // T
LR = 32
FC1, FC2 = 768, 384
bf16, f32 = jnp.bfloat16, jnp.float32
NN = (((1,), (0,)), ((), ()))
NT = (((1,), (1,)), ((), ()))
TN = (((0,), (0,)), ((), ()))

ROWS = [(0, 144), (112, 272), (240, 400), (368, 528), (496, 576)]
A_TERMS = [((0, 0), (1, 1), 1), ((1, 0), (1, 1), 1), ((0, 0), None, 0), ((1, 1), None, 0),
           ((0, 0), (0, 1), 1), ((1, 0), (0, 0), -1), ((0, 1), (1, 1), -1)]
B_TERMS = [((0, 0), (1, 1), 1), ((0, 0), None, 0), ((0, 1), (1, 1), -1), ((1, 0), (0, 0), -1),
           ((1, 1), None, 0), ((0, 0), (0, 1), 1), ((1, 0), (1, 1), 1)]


def _dot(a, b, dims=NN):
    return lax.dot_general(a, b, dims, preferred_element_type=f32)


def _dot576(w, x):
    return _dot(w[0:512, :], x[0:512, :], TN) + _dot(w[512:D, :], x[512:D, :], TN)


def _phi(t):
    return jnp.where(t > 0, t + 1.0, jnp.exp(t)) + 1e-6


def _relu2(x):
    r = jnp.maximum(x, 0.0)
    return r * r


def _head_of(i):
    return (i * 3641) >> 16


def _madd(X, Y, s=1):
    return {k: (X[k] + Y[k] if s > 0 else X[k] - Y[k]) for k in X}


def _operands(X, terms):
    return [X[p] if q is None else (X[p] + X[q] if s > 0 else X[p] - X[q]) for p, q, s in terms]


def _combine(M, L):
    if L == 0:
        return {(0, 0): M[0]}
    n = 7 ** (L - 1)
    m = [_combine(M[j * n:(j + 1) * n], L - 1) for j in range(7)]
    C11 = _madd(_madd(_madd(m[0], m[3]), m[4], -1), m[6])
    C12 = _madd(m[2], m[4])
    C21 = _madd(m[1], m[3])
    C22 = _madd(_madd(_madd(m[0], m[1], -1), m[2]), m[5])
    h = 2 ** (L - 1)
    out = {}
    for a, b, X in ((0, 0, C11), (0, 1, C12), (1, 0, C21), (1, 1, C22)):
        for (i, j), v in X.items():
            out[(a * h + i, b * h + j)] = v
    return out


def _tile(v, rows, cols):
    v = jnp.concatenate([v] * (cols // 128), axis=1) if cols > 128 else v
    return jnp.concatenate([v] * (rows // 8), axis=0) if rows > 8 else v


def _mix(a, b):
    out, ia, ib, na, nb = [], 0, 0, len(a), len(b)
    while ia < na or ib < nb:
        if ib >= nb or (ia < na and ia * nb <= ib * na):
            out.append(a[ia])
            ia += 1
        else:
            out.append(b[ib])
            ib += 1
    return out


def _part(lst, i, n):
    return lst[i * len(lst) // n:(i + 1) * len(lst) // n]


def _run(res, tasks, lo=0.0, hi=1.0):
    rows, cols = res.shape
    nr, nc = rows // 8, cols // 128
    for i, task in enumerate(tasks):
        p = int((lo + (hi - lo) * i / len(tasks)) * nr * nc)
        c, r = divmod(min(p, nr * nc - 1), nr)
        task(jnp.maximum(jnp.minimum(res[8 * r:8 * r + 8, 128 * c:128 * c + 128], 0.0), 0.0))


def _ones_rows(n):
    return jnp.where(lax.broadcasted_iota(jnp.int32, (16, n), 0) == 0, 1.0, 0.0).astype(bf16)


def _kernel(x_hbm, wqkv_hbm, wo_hbm, w1_hbm, b1_hbm, w2_hbm, b2_hbm, o_hbm,
            x_v, wq_v, wk_v, wv_v, wo_v, w1_v, w2_v, b1_v, b2_v, a1_v, a1b_v, a2_v,
            xn_v, pq_v, z_v, b2c_v, g_v, wa_v, h_v, hs_v, hs2_v, ht_v, rs_v, o_v,
            xsem, wsem, osem, bsem):
    def cpx(i, lo, n):
        return pltpu.make_async_copy(x_hbm.at[:, pl.ds(lo, n)], x_v.at[:, pl.ds(lo, n)], xsem.at[i])
    cp_x0, cp_x1, cp_x2 = cpx(0, 0, T), cpx(1, T, T), cpx(2, 2 * T, S - 2 * T)
    cp_wk = pltpu.make_async_copy(wqkv_hbm.at[:, pl.ds(512, 640)], wk_v, wsem.at[0])
    cp_wq = pltpu.make_async_copy(wqkv_hbm.at[:, pl.ds(0, 512)], wq_v, wsem.at[1])
    cp_wv = pltpu.make_async_copy(wqkv_hbm.at[:, pl.ds(2 * D, D)], wv_v, wsem.at[2])
    cp_wo = pltpu.make_async_copy(wo_hbm, wo_v, wsem.at[3])
    cp_w1 = [pltpu.make_async_copy(w1_hbm.at[:, pl.ds(c, FQ)], w1_v.at[pl.ds(0, D), pl.ds(c, FQ)], wsem.at[4 + i])
             for i, c in enumerate((0, FH, FQ, FH + FQ))]
    cp_w2 = pltpu.make_async_copy(w2_hbm, w2_v, wsem.at[8])
    cp_b1 = pltpu.make_async_copy(b1_hbm, b1_v, wsem.at[9])
    cp_b2 = pltpu.make_async_copy(b2_hbm, b2_v, wsem.at[10])

    def out_copy(t, blk=None):
        if blk is None:
            sl = pl.ds(t * T, T)
            return pltpu.make_async_copy(o_v.at[:, sl], o_hbm.at[:, sl], osem.at[t])
        rows, cols = pl.ds(DHF * (blk // 2), DHF), pl.ds(t * T + TH * (blk % 2), TH)
        return pltpu.make_async_copy(o_v.at[rows, cols], o_hbm.at[rows, cols], osem.at[NTI - 1 + blk])

    def barrier():
        pl.semaphore_signal(bsem, 1)
        pl.semaphore_wait(bsem, 1)

    def var_tasks(load, st):
        n = D // LR

        def piece(i):
            def f(g):
                mg = jnp.concatenate([st['m'] + _tile(g, 8, T)] * (LR // 8), axis=0)
                c = load(i * LR) - mg
                c = c * c
                st['acc'] = c if i == 0 else st['acc'] + c
                if i == n - 1:
                    v = jnp.sum(st['acc'], axis=0, keepdims=True) * (1.0 / D)
                    st['rstd'] = jnp.broadcast_to(lax.rsqrt(v + 1e-5), (8, T))
            return f
        return [piece(i) for i in range(n)]

    def ln1_tasks(t):
        sl = pl.ds(t * T, T)
        st = {}
        n = D // LR

        def load(r):
            return x_v[r:r + LR, sl].astype(f32)

        def mean_piece(i):
            def f(g):
                c = load(i * LR)
                gt = _tile(g, LR, T)
                st['acc'] = (c + gt) if i == 0 else (st['acc'] + gt) + c
                if i == n - 1:
                    m = jnp.sum(st['acc'], axis=0, keepdims=True) * (1.0 / D)
                    st['m'] = jnp.broadcast_to(m, (8, T))
            return f

        def norm_piece(i):
            def f(g):
                mg = jnp.concatenate([st['m'] + _tile(g, 8, T)] * (LR // 8), axis=0)
                rs = jnp.concatenate([st['rstd']] * (LR // 8), axis=0)
                r = i * LR
                xn_v[r:r + LR, sl] = ((load(r) - mg) * rs).astype(bf16)
                if i == n - 1:
                    xn_v[D:DA, sl] = _ones_rows(T)
            return f
        return [mean_piece(i) for i in range(n)] + var_tasks(load, st) + [norm_piece(i) for i in range(n)]

    def weight_tasks(which, lo, hi):
        src, dst, rows = (w1_v, a1_v, 256) if which == 1 else (w2_v, a2_v, DHF)
        tasks = []
        for c0 in range(lo, hi, 256):
            cw = min(256, hi - c0)
            ca, cb = slice(c0, c0 + cw), slice(FH + c0, FH + c0 + cw)
            for r in range(0, rows, 16):
                ra, rb = slice(r, r + 16), slice(rows + r, rows + r + 16)

                def f(g, ra=ra, rb=rb, ca=ca, cb=cb, cw=cw):
                    gt = _tile(g, 16, cw)
                    A11 = src[ra, ca].astype(f32) + gt
                    A22 = src[rb, cb].astype(f32) + gt
                    if which == 1:
                        A12, A21 = src[rb, ca].astype(f32), src[ra, cb].astype(f32)
                    else:
                        A12, A21 = src[ra, cb].astype(f32), src[rb, ca].astype(f32)
                    for j, a in enumerate([A11 + A22, A21 + A22, A11 + A12, A21 - A11, A12 - A22]):
                        dst[j, ra, ca] = a.astype(bf16)
                tasks.append(f)
        return tasks

    def weight_tasks2():
        tasks = []
        for c0 in range(0, FQ, 128):
            for r in range(0, 128, 16):
                for j1, (P, Q, sg) in enumerate(A_TERMS):
                    def f(g, c0=c0, r=r, j1=j1, P=P, Q=Q, sg=sg):
                        gt = _tile(g, 16, 128)

                        def blk(sb, i, j):
                            a, b = 2 * sb[0] + i, 2 * sb[1] + j
                            return w1_v[128 * b + r:128 * b + r + 16, a * FQ + c0:a * FQ + c0 + 128]
                        raw = {(i, j): blk(P, i, j) for i in range(2) for j in range(2)}
                        X = {k: (v.astype(f32) + gt if k[0] == k[1] else v.astype(f32)) for k, v in raw.items()}
                        if Q is not None:
                            X = _madd(X, {(i, j): blk(Q, i, j).astype(f32) for i in range(2) for j in range(2)}, sg)
                        for j2, v in enumerate(_operands(X, A_TERMS)):
                            if Q is None and j2 in (2, 3):
                                v = raw[(0, 0)] if j2 == 2 else raw[(1, 1)]
                            a1b_v[7 * j1 + j2, r:r + 16, c0:c0 + 128] = v.astype(bf16)
                    tasks.append(f)
        return tasks

    def fold():
        parts = []
        for j, (r0, r1) in enumerate(ROWS):
            c0, c1 = j * 128, min((j + 1) * 128, D)
            kv = _dot(g_v[r0:r1, 0:D].astype(bf16), wv_v[:, c0:c1])
            ri = lax.broadcasted_iota(jnp.int32, (r1 - r0, c1 - c0), 0) + r0
            ci = lax.broadcasted_iota(jnp.int32, (r1 - r0, c1 - c0), 1) + c0
            kvm = jnp.where(_head_of(ri) == _head_of(ci), kv, 0.0).astype(bf16)
            parts.append(_dot(kvm, wo_v[c0:c1, :]))
        for j, (r0, r1) in enumerate(ROWS):
            lo = r0 if j == 0 else ROWS[j - 1][1]
            hi = r1 if j == 4 else ROWS[j + 1][0]
            wa_v[lo:hi, :] = parts[j][lo - r0:hi - r0, :].astype(bf16)
            if j < 4:
                n0 = ROWS[j + 1][0]
                wa_v[hi:r1, :] = (parts[j][hi - r0:, :] + parts[j + 1][0:r1 - n0, :]).astype(bf16)

    sub8 = lax.broadcasted_iota(jnp.int32, (8, 128), 0)

    def qproj(t):
        sl = pl.ds(t * T, T)
        q = _dot576(wq_v, xn_v[0:D, sl])
        for l in range(T // 128):
            cl = pl.ds(t * T + l * 128, 128)
            for g in range(4):
                if g < 3:
                    pq = _phi(q[144 * g:144 * g + 144, 128 * l:128 * l + 128])
                else:
                    pq = jnp.concatenate([_phi(q[432:512, 128 * l:128 * l + 128]), pq_v[512:D, cl].astype(f32)], axis=0)
                pz = pq * z_v[144 * g:144 * g + 144, :]
                rden = []
                for h in range(8):
                    a, o = divmod(h * DH, 8)
                    first, last = pz[8 * a:8 * a + 8, :], pz[8 * a + 16:8 * a + 24, :]
                    tt = pz[8 * a + 8:8 * a + 16, :]
                    tt = tt + (first if o == 0 else jnp.where(sub8 >= o, first, 0.0))
                    tt = tt + (last if o == 6 else jnp.where(sub8 < o + 2, last, 0.0))
                    den = jnp.sum(tt, axis=0, keepdims=True) + 1e-6
                    r0 = pl.reciprocal(den, approx=True)
                    rden.append(r0 * (2.0 - den * r0))
                outs = []
                for i in range(18):
                    h0, h1 = (8 * i) // DH, (8 * i + 7) // DH
                    blk = pq[8 * i:8 * i + 8, :]
                    if h0 == h1:
                        outs.append(blk * rden[h0])
                    else:
                        outs.append(blk * jnp.where(sub8 < h1 * DH - 8 * i, rden[h0], rden[h1]))
                pq_v[144 * g:144 * g + 144, cl] = jnp.concatenate(outs, axis=0).astype(bf16)

    def attn_out(t):
        sl = pl.ds(t * T, T)
        att = _dot576(wa_v, pq_v[:, sl])
        acc = None
        for r in range(0, D, LR):
            c = x_v[r:r + LR, sl].astype(f32) + att[r:r + LR, :]
            h_v[r:r + LR, sl] = c
            acc = c if acc is None else acc + c
        st = {'m': jnp.broadcast_to(jnp.sum(acc, axis=0, keepdims=True) * (1.0 / D), (8, T))}
        tasks = var_tasks(lambda r: h_v[r:r + LR, sl], st)

        def stats(g):
            return (jnp.concatenate([st['m'] + _tile(g, 8, T)] * 2, axis=0),
                    jnp.concatenate([st['rstd']] * 2, axis=0))

        def one_level(r):
            def f(g):
                mg, rs = stats(g)
                a = (h_v[r:r + 16, sl] - mg) * rs
                b = (h_v[256 + r:256 + r + 16, sl] - mg) * rs
                X = {(0, 0): a[:, :TH], (0, 1): a[:, TH:], (1, 0): b[:, :TH], (1, 1): b[:, TH:]}
                for j, c in enumerate(_operands(X, B_TERMS)):
                    hs_v[j, r:r + 16, :] = c.astype(bf16)
            return f

        def two_level(r, j1):
            P, Q, sg = B_TERMS[j1]

            def f(g):
                mg, rs = stats(g)

                def blk(sb, i, j):
                    a, b = 2 * sb[0] + i, 2 * sb[1] + j
                    cs = slice(128 * b, 128 * b + 128)
                    return (h_v[128 * a + r:128 * a + r + 16, pl.ds(t * T + 128 * b, 128)] - mg[:, cs]) * rs[:, cs]
                X = {(i, j): blk(P, i, j) for i in range(2) for j in range(2)}
                if Q is not None:
                    X = _madd(X, {(i, j): blk(Q, i, j) for i in range(2) for j in range(2)}, sg)
                for j2, v in enumerate(_operands(X, B_TERMS)):
                    hs2_v[7 * j1 + j2, r:r + 16, pl.ds(t * 128, 128)] = v.astype(bf16)
            return f

        def tail(r):
            def f(g):
                mg, rs = stats(g)
                ht_v[r - 512:r - 512 + 16, sl] = ((h_v[r:r + 16, sl] - mg) * rs).astype(bf16)
                if r + 16 == D:
                    ht_v[64:80, sl] = _ones_rows(T)
            return f
        if t == 0:
            tasks += [one_level(r) for r in range(0, 256, 16)]
        else:
            tasks += [two_level(r, j1) for r in range(0, 128, 16) for j1 in range(7)]
        return att, tasks + [tail(r) for r in range(512, D, 16)]

    def biases():
        r16 = lax.broadcasted_iota(jnp.int32, (16, 128), 0)
        b1f = b1_v[...].astype(f32)
        for i in range(F // 128):
            w1_v[D:DA, i * 128:(i + 1) * 128] = jnp.where(r16 == 0, b1f[i:i + 1, :], 0.0).astype(bf16)
        b2row = b2_v[...].reshape(1, D).astype(f32)
        r16d = lax.broadcasted_iota(jnp.int32, (16, D), 0)
        b2t = jnp.where(r16d == 0, b2row, 0.0).astype(bf16)
        b2c_v[...] = _dot(b2t, jnp.ones((16, 128), bf16), TN)

    def mlp1_one_level(t, f0, fill):
        sl = pl.ds(t * T, T)
        fa, fb = slice(f0, f0 + FC1), slice(FH + f0, FH + f0 + FC1)
        lhs = [a1_v[0, :, fa], a1_v[1, :, fa], w1_v[0:256, fa], w1_v[256:512, fb],
               a1_v[2, :, fa], a1_v[3, :, fa], a1_v[4, :, fa]]
        M = [_dot(lhs[j], hs_v[j], TN) for j in range(7)]
        htv = ht_v[:, sl]
        ta = _dot(w1_v[512:DA, fa], htv, TN)
        tb = _dot(w1_v[512:DA, fb], htv, TN)
        C = _combine(M, 1)
        R = {(0, 0): _relu2(C[(0, 0)] + ta[:, :TH]), (0, 1): _relu2(C[(0, 1)] + ta[:, TH:]),
             (1, 0): _relu2(C[(1, 0)] + tb[:, :TH]), (1, 1): _relu2(C[(1, 1)] + tb[:, TH:])}
        for j, v in enumerate(_operands(R, B_TERMS)):
            rs_v[j, fa, :] = v.astype(bf16)
        for j in range(7):
            _run(M[j], _part(fill, j, 7))

    def mlp1_two_level(t, f0, fill):
        sl = pl.ds(t * T, T)
        M = [_dot(a1b_v[j, :, f0:f0 + FC2], hs2_v[j, :, pl.ds(t * 128, 128)], TN) for j in range(49)]
        C = _combine(M, 2)
        htv = ht_v[:, sl]
        R = {}
        for a in range(4):
            tl = _dot(w1_v[512:DA, a * FQ + f0:a * FQ + f0 + FC2], htv, TN)
            for b in range(4):
                R[(a, b)] = _relu2(C[(a, b)] + tl[:, 128 * b:128 * b + 128])
        for sub in range(2):
            B = {(a, b): jnp.concatenate([R[(2 * a + sub, 2 * b)], R[(2 * a + sub, 2 * b + 1)]], axis=1)
                 for a in range(2) for b in range(2)}
            fo = sub * FQ + f0
            for j, v in enumerate(_operands(B, B_TERMS)):
                rs_v[j, fo:fo + FC2, :] = v.astype(bf16)
        for j in range(49):
            _run(M[j], _part(fill, j, 49))

    def mlp2(t, fill):
        lhs = [a2_v[0], a2_v[1], w2_v[0:DHF, 0:FH], w2_v[DHF:D, FH:F], a2_v[2], a2_v[3], a2_v[4]]
        last = t == NTI - 1
        b2a = jnp.concatenate([b2c_v[0:DHF, :]] * (TH // 128), axis=1)
        b2b = jnp.concatenate([b2c_v[DHF:D, :]] * (TH // 128), axis=1)
        sa, sb = pl.ds(t * T, TH), pl.ds(t * T + TH, TH)
        M = [None] * 7
        cuts = list(range(0, FH, 512)) + [FH] if fill else [0, FH]
        nslot = 7 * (len(cuts) - 1)
        slot = [0]

        def prod(*js):
            for j in js:
                acc = None
                for k0, k1 in zip(cuts[:-1], cuts[1:]):
                    part = _dot(lhs[j][:, k0:k1], rs_v[j, k0:k1, :])
                    acc = part if acc is None else acc + part
                    _run(part, _part(fill, slot[0], nslot))
                    slot[0] += 1
                M[j] = acc
        prod(2, 4)
        o_v[0:DHF, sb] = (h_v[0:DHF, sb] + b2a + (M[2] + M[4])).astype(bf16)
        if last:
            out_copy(t, 1).start()
        prod(1, 3)
        o_v[DHF:D, sa] = (h_v[DHF:D, sa] + b2b + (M[1] + M[3])).astype(bf16)
        if last:
            out_copy(t, 2).start()
        prod(0, 6)
        o_v[0:DHF, sa] = (h_v[0:DHF, sa] + b2a + (M[0] + M[3] - M[4] + M[6])).astype(bf16)
        if last:
            out_copy(t, 0).start()
        prod(5)
        o_v[DHF:D, sb] = (h_v[DHF:D, sb] + b2b + (M[0] - M[1] + M[2] + M[5])).astype(bf16)
        out_copy(t, 3 if last else None).start()

    cp_x0.start()
    cp_wk.start()
    cp_x0.wait()
    cp_x1.start()
    for task in ln1_tasks(0):
        task(jnp.zeros((8, 128), f32))
    cp_wk.wait()
    cp_x2.start()
    for t in range(NTI):
        sl = pl.ds(t * T, T)
        a1 = []
        if t == 2:
            cp_w1[0].wait()
            cp_w1[1].wait()
            cp_w2.start()
            a1 = weight_tasks(1, 0, FQ)
        if t == 3:
            cp_w1[2].wait()
            cp_w1[3].wait()
            a1 = weight_tasks(1, FQ, FH)
        kq = _dot576(wk_v, xn_v[0:D, sl])
        pkq = _phi(kq)
        pq_v[512:D, sl] = pkq[0:64, :].astype(bf16)
        pk = pkq[64:640, :].astype(bf16)
        ln = ln1_tasks(t + 1) if t + 1 < NTI else []
        if t == 0:
            cp_x1.wait()
            cp_w1[0].start()
            cp_w1[1].start()
        elif t == 1:
            cp_x2.wait()
            for cp in (cp_w1[2], cp_w1[3], cp_wv, cp_wo, cp_wq, cp_b1, cp_b2):
                cp.start()
        if t >= 2:
            _run(kq, _mix(_part(ln, 0, 2), _part(a1, 0, 2)))
            ln = _mix(_part(ln, 1, 2), _part(a1, 1, 2))
        g = _dot(pk, xn_v[:, sl], NT)
        _run(g[:, 0:512], ln)
        if t == 0:
            g_v[...] = g
        else:
            g_v[...] += g
    for cp in (cp_wv, cp_wo, cp_wq, cp_b1, cp_b2):
        cp.wait()

    z_v[...] = jnp.broadcast_to(g_v[:, D:D + 1], (D, 128))
    fold()
    qproj(0)
    qproj(1)
    biases()
    a2 = weight_tasks(2, 0, FH)
    n2 = int(len(a2) * 0.4)
    cp_w2.wait()
    att, ln2_first = attn_out(0)
    _run(att, a2[:n2 // 2])
    att, ln2 = attn_out(1)
    _run(att, ln2_first, 0.0, 0.8)
    _run(att, a2[n2 // 2:n2])
    a2 = a2[n2:]
    barrier()

    for t in range(NTI):
        chunks = range(0, FH, FC1) if t == 0 else range(0, FQ, FC2)
        for ci, f0 in enumerate(chunks):
            if 0 < t < NTI - 1 and ci == 0:
                _, ln2 = attn_out(t + 1)
            if t + 2 < NTI and ci == 2:
                qproj(t + 2)
            fill = _mix(_part(a2, ci, 3) if t == 0 else [], _part(ln2, ci, 3) if t < NTI - 1 else [])
            (mlp1_one_level if t == 0 else mlp1_two_level)(t, f0, fill)
        mlp2(t, weight_tasks2() if t == 0 else [])
        barrier()

    for t in range(NTI - 1):
        out_copy(t).wait()
    for blk in range(4):
        out_copy(NTI - 1, blk).wait()


@jax.jit
def pallas_sequential_preLN__linear_attn_block__dense_activation_squared_relu__prompt_kernel(
    A_x: jax.Array,
    A_wqkv: jax.Array,
    A_wo: jax.Array,
    B_x: jax.Array,
    B_w1: jax.Array,
    B_b1: jax.Array,
    B_w2: jax.Array,
    B_b2: jax.Array,
):
    del B_x
    anyspec = pl.BlockSpec(memory_space=pl.ANY)
    out = pl.pallas_call(
        _kernel,
        out_shape=jax.ShapeDtypeStruct((D, S), bf16),
        in_specs=[anyspec] * 7,
        out_specs=anyspec,
        scratch_shapes=[
            pltpu.VMEM((D, S), bf16),
            pltpu.VMEM((D, 512), bf16),
            pltpu.VMEM((D, 640), bf16),
            pltpu.VMEM((D, D), bf16),
            pltpu.VMEM((D, D), bf16),
            pltpu.VMEM((DA, F), bf16),
            pltpu.VMEM((D, F), bf16),
            pltpu.VMEM((F // 128, 128), bf16),
            pltpu.VMEM((D,), bf16),
            pltpu.VMEM((5, 256, FH), bf16),
            pltpu.VMEM((49, 128, FQ), bf16),
            pltpu.VMEM((5, DHF, FH), bf16),
            pltpu.VMEM((DA, S), bf16),
            pltpu.VMEM((D, S), bf16),
            pltpu.VMEM((D, 128), f32),
            pltpu.VMEM((D, 128), f32),
            pltpu.VMEM((D, DA), f32),
            pltpu.VMEM((D, D), bf16),
            pltpu.VMEM((D, S), f32),
            pltpu.VMEM((7, 256, TH), bf16),
            pltpu.VMEM((49, 128, S // 4), bf16),
            pltpu.VMEM((80, S), bf16),
            pltpu.VMEM((7, FH, TH), bf16),
            pltpu.VMEM((D, S), bf16),
            pltpu.SemaphoreType.DMA((3,)),
            pltpu.SemaphoreType.DMA((11,)),
            pltpu.SemaphoreType.DMA((NTI + 3,)),
            pltpu.SemaphoreType.REGULAR,
        ],
        compiler_params=pltpu.CompilerParams(vmem_limit_bytes=110 * 2**20),
        name="preln_linear_attn_relu2_mlp",
    )(A_x.reshape(S, D).T, A_wqkv, A_wo, B_w1, B_b1.reshape(F // 128, 128), B_w2.T, B_b2)
    return out.T.reshape(1, S, D)
```
